```python
import jax
import jax.numpy as jnp

def _softmax(x, axis=-1):
    return jax.nn.softmax(x, axis=axis)

def _gelu(x):
    return jax.nn.gelu(x, approximate=True)

def _silu(x):
    return jax.nn.silu(x)

def _sigmoid(x):
    return jax.nn.sigmoid(x)

def _layernorm(x, axis=-1, eps=1e-05):
    m = jnp.mean(x, axis=axis, keepdims=True)
    v = jnp.var(x, axis=axis, keepdims=True)
    return (x - m) / jnp.sqrt(v + eps)

def _scatter_add(tgt, idx, src, axis=0):
    return tgt.at[idx].add(src)

def _segment_sum(src, seg, n):
    return jax.ops.segment_sum(src, seg, n)

class _Rng:

    def __init__(self, key):
        self._k = key

    def _next(self):
        self._k, sub = jax.random.split(self._k)
        return sub

    def normal(self, shape):
        return jax.random.normal(self._next(), shape, dtype=jnp.bfloat16)

    def randint(self, lo, hi, shape):
        return jax.random.randint(self._next(), shape, lo, hi, dtype=jnp.int32)

    def uniform(self, shape, lo=0.0, hi=1.0):
        return jax.random.uniform(self._next(), shape, jnp.bfloat16, lo, hi)

    def permutation(self, n):
        return jax.random.permutation(self._next(), n)
kernel_name = 'adaLN_cond__sliding_block_cached__dense_activation_gelu__decode'

def setup_inputs():
    _rng = _Rng(jax.random.key(int.from_bytes(__import__("os").urandom(4), "little")))
    _w = lambda a: (lambda t: t.astype(jnp.bfloat16) if jnp.issubdtype(t.dtype, jnp.floating) else t)(jnp.asarray(a))

    def _A_setup():
        B, Sq, D = (4, 1, 640)
        Hq, Hkv, Sk, Dh = (32, 32, 8192, 128)
        assert Hq % Hkv == 0, (Hq, Hkv)
        return {'x': _w((lambda *s: _rng.normal(s) * 0.05)(B, Sq, D)), 'k_cache': _w((lambda *s: _rng.normal(s) * 0.05)(B, Hkv, Sk, Dh)), 'v_cache': _w((lambda *s: _rng.normal(s) * 0.05)(B, Hkv, Sk, Dh)), 'wq': _w((lambda *s: _rng.normal(s) * 0.05)(D, Hq * Dh) * D ** (-0.5)), 'wo': _w((lambda *s: _rng.normal(s) * 0.05)(Hq * Dh, D) * (Hq * Dh) ** (-0.5))}
    _A_in = _A_setup()

    def _B_setup():
        B, S, D, F = (4, 1, 640, 1728)
        return {'x': _w((lambda *s: _rng.normal(s) * 0.05)(B, S, D)), 'w1': _w((lambda *s: _rng.normal(s) * 0.05)(D, F) * D ** (-0.5)), 'b1': _w((lambda *s: _rng.normal(s) * 0.05)(F) * 0.01), 'w2': _w((lambda *s: _rng.normal(s) * 0.05)(F, D) * F ** (-0.5)), 'b2': _w((lambda *s: _rng.normal(s) * 0.05)(D) * 0.01)}
    _B_in = _B_setup()
    return {'A_x': _A_in['x'], 'A_k_cache': _A_in['k_cache'], 'A_v_cache': _A_in['v_cache'], 'A_wq': _A_in['wq'], 'A_wo': _A_in['wo'], 'B_x': _B_in['x'], 'B_w1': _B_in['w1'], 'B_b1': _B_in['b1'], 'B_w2': _B_in['w2'], 'B_b2': _B_in['b2'], 'c': _w((lambda *s: _rng.normal(s) * 0.05)(4, 640)), 'w_mod': _w((lambda *s: _rng.normal(s) * 0.05)(640, 6 * 640) * 640 ** (-0.5))}

def reference(A_x, A_k_cache, A_v_cache, A_wq, A_wo, B_x, B_w1, B_b1, B_w2, B_b2, c, w_mod):

    def _A_ref(x, k_cache, v_cache, wq, wo):
        B, Sq, D = x.shape
        Hq, Dh = (32, 128)
        Hkv, Sk = (k_cache.shape[1], k_cache.shape[2])
        W = min(4096, max(256, Sk // 4))
        rep = Hq // Hkv
        q = (lambda x, *d: x.transpose(*d))((x @ wq).reshape(B, Sq, Hq, Dh), 0, 2, 1, 3)
        k = jnp.repeat(k_cache[:, :, Sk - W:, :], rep, axis=1)
        v = jnp.repeat(v_cache[:, :, Sk - W:, :], rep, axis=1)
        scores = jnp.einsum('bhqd,bhkd->bhqk', q, k) * Dh ** (-0.5)
        p = _softmax(scores, axis=-1)
        o = jnp.einsum('bhqk,bhkd->bhqd', p, v)
        return (lambda x, *d: x.transpose(*d))(o, 0, 2, 1, 3).reshape(B, Sq, Hq * Dh) @ wo

    def _B_ref(x, w1, b1, w2, b2):
        h = jnp.einsum('bsd,df->bsf', x, w1) + b1
        h = _gelu(h)
        return jnp.einsum('bsf,fd->bsd', h, w2) + b2
    x = A_x
    mod = (_silu(c) @ w_mod).reshape(c.shape[0], 6, 1, -1)
    sa, ca, ga, sb, cb, gb = (mod[:, 0].copy(), mod[:, 1].copy(), mod[:, 2].copy(), mod[:, 3].copy(), mod[:, 4].copy(), mod[:, 5].copy())
    h = _layernorm(x, axis=-1) * (1 + ca) + sa
    x = x + ga * _A_ref(h, A_k_cache, A_v_cache, A_wq, A_wo)
    h = _layernorm(x, axis=-1) * (1 + cb) + sb
    x = x + gb * _B_ref(h, B_w1, B_b1, B_w2, B_b2)
    return x
```

```python
import jax
import jax.numpy as jnp
from jax import lax
import jax.experimental.pallas as pl
import jax.experimental.pallas.tpu as pltpu

F32 = jnp.float32
BF16 = jnp.bfloat16
_NT = (((1,), (1,)), ((), ()))

KV_ROWS = 128
MOD_CH = (16, 640)
WQ_CH = (16, 512)
W_ROWS = 16
Q_PARTS = 2
W2_PARTS = (512, 512, 512, 192)


def _layernorm(x):
    m = jnp.mean(x, axis=-1, keepdims=True)
    d = x - m
    v = jnp.mean(d * d, axis=-1, keepdims=True)
    return d / jnp.sqrt(v + 1e-05)


def _block_kernel(x_hbm, c_hbm, wmod_hbm, wq_hbm, k_hbm, v_hbm, wo_hbm, w1t_hbm, b1_hbm, w2_hbm, b2_hbm,
                  out_ref,
                  x_v, c_v, b1_v, b2_v, wmod_v, wq_v, wo_v, w1_v, w2_v, kbuf, vbuf, q_scr, o_scr,
                  ksem, vsem, ssem, msem, qsem, osem, w1sem, w2sem):
    B, D = x_v.shape
    _, H, Sk, Dh = k_hbm.shape
    W = kbuf.shape[1]
    F = w1_v.shape[0]
    HD = H * Dh
    scale = Dh ** (-0.5)

    def stream(src, dst, sem, r0, nr, c0, nc, ch):
        cr, cw = ch
        half = nr // 2
        assert nr % 2 == 0 and half % cr == 0 and r0 % cr == 0 and nc % cw == 0

        def body(i, carry):
            for cc in range(c0, c0 + nc, cw):
                for p in range(2):
                    r = pl.multiple_of(r0 + p * half + i * cr, cr)
                    pltpu.make_async_copy(src.at[pl.ds(r, cr), pl.ds(cc, cw)],
                                          dst.at[pl.ds(r, cr), pl.ds(cc, cw)], sem).start(priority=p)
            return carry

        lax.fori_loop(0, half // cr, body, 0)

    def wait(dst, sem):
        pltpu.make_async_copy(dst, dst, sem).wait()

    def fill(src, buf, sem, b, h):
        hs = W // KV_ROWS // 2
        for i in range(hs):
            for p in range(2):
                r = (p * hs + i) * KV_ROWS
                pltpu.make_async_copy(src.at[b, h, pl.ds(Sk - W + r, KV_ROWS), :],
                                      buf.at[b, pl.ds(r, KV_ROWS), :], sem.at[b]).start(priority=p)

    def prime(b0, b1):
        def body(b, carry):
            fill(k_hbm, kbuf, ksem, b, 0)
            fill(v_hbm, vbuf, vsem, b, 0)
            return carry

        lax.fori_loop(b0, b1, body, 0)

    pltpu.make_async_copy(c_hbm, c_v, ssem.at[0]).start(priority=0)
    pltpu.make_async_copy(x_hbm, x_v, ssem.at[1]).start(priority=1)
    stream(wmod_hbm, wmod_v, msem.at[0], 0, D, 0, 2 * D, MOD_CH)
    qn = HD // Q_PARTS
    stream(wq_hbm, wq_v, qsem.at[0], 0, D, 0, qn, WQ_CH)

    wait(c_v, ssem.at[0])
    wait(x_v, ssem.at[1])
    cf = c_v[...].astype(F32)
    sc = (cf * jax.nn.sigmoid(cf)).astype(BF16)
    x = x_v[...].astype(F32)
    xn = _layernorm(x)
    wait(wmod_v.at[:, pl.ds(0, 2 * D)], msem.at[0])
    mod_a = jnp.dot(sc, wmod_v[:, 0:2 * D], preferred_element_type=F32)
    sa, ca = mod_a[:, 0:D], mod_a[:, D:2 * D]
    ha = (xn * (1.0 + ca) + sa).astype(BF16)

    for i in range(Q_PARTS):
        if i + 1 < Q_PARTS:
            stream(wq_hbm, wq_v, qsem.at[i + 1], 0, D, (i + 1) * qn, qn, WQ_CH)
        else:
            prime(0, B // 2)
        wait(wq_v.at[:, pl.ds(i * qn, qn)], qsem.at[i])
        q = jnp.dot(ha, wq_v[:, i * qn:(i + 1) * qn], preferred_element_type=F32)
        for h in range(qn // Dh):
            q_scr[i * (qn // Dh) + h] = q[:, h * Dh:(h + 1) * Dh]
    prime(B // 2, B)
    pltpu.make_async_copy(b1_hbm, b1_v, ssem.at[2]).start(priority=0)
    pltpu.make_async_copy(b2_hbm, b2_v, ssem.at[3]).start(priority=1)

    row = lax.broadcasted_iota(jnp.int32, (B, Dh), 0)

    def head(h, last):
        qh = q_scr[h].astype(BF16)
        acc = jnp.zeros((B, Dh), F32)
        n = HD // (2 * B)
        for b in range(B):
            wait(kbuf.at[b], ksem.at[b])
            s = lax.dot_general(qh, kbuf[b], _NT, preferred_element_type=F32) * scale
            if last:
                stream(wo_hbm, wo_v, osem, 2 * b * n, n, 0, D, (W_ROWS, D))
            else:
                fill(k_hbm, kbuf, ksem, b, h + 1)
            m = jnp.max(s, axis=-1, keepdims=True)
            p = jnp.exp(s - m)
            l = jnp.sum(p, axis=-1, keepdims=True)
            wait(vbuf.at[b], vsem.at[b])
            o = jnp.dot(p.astype(BF16), vbuf[b], preferred_element_type=F32)
            if last:
                stream(wo_hbm, wo_v, osem, (2 * b + 1) * n, n, 0, D, (W_ROWS, D))
            else:
                fill(v_hbm, vbuf, vsem, b, h + 1)
            acc = jnp.where(row == b, o / l, acc)
        o_scr[h] = acc

    def head_body(h, carry):
        head(h, False)
        return carry

    lax.fori_loop(0, H - 1, head_body, 0)
    head(H - 1, True)

    stream(wmod_hbm, wmod_v, msem.at[1], 0, D, 2 * D, 4 * D, MOD_CH)
    o_all = jnp.concatenate([o_scr[h] for h in range(H)], axis=-1).astype(BF16)
    wait(wo_v, osem)
    attn = jnp.dot(o_all, wo_v[...], preferred_element_type=F32)

    stream(w1t_hbm, w1_v, w1sem, 0, F, 0, D, (W_ROWS, D))
    wait(wmod_v.at[:, pl.ds(2 * D, 4 * D)], msem.at[1])
    mod_b = jnp.dot(sc, wmod_v[:, 2 * D:6 * D], preferred_element_type=F32)
    ga, sb, cb, gb = (mod_b[:, i * D:(i + 1) * D] for i in range(4))
    x1 = x + ga * attn
    hb = (_layernorm(x1) * (1.0 + cb) + sb).astype(BF16)

    starts = [sum(W2_PARTS[:i]) for i in range(len(W2_PARTS))]
    for i, (r, n) in enumerate(zip(starts, W2_PARTS)):
        stream(w2_hbm, w2_v, w2sem.at[i], r, n, 0, D, (W_ROWS, D))
    wait(b1_v, ssem.at[2])
    wait(b2_v, ssem.at[3])
    b1 = b1_v[...].astype(F32).reshape(1, F)
    b2 = b2_v[...].astype(F32).reshape(1, D)
    wait(w1_v, w1sem)
    u = lax.dot_general(hb, w1_v[...], _NT, preferred_element_type=F32) + b1
    u = jax.nn.gelu(u, approximate=True).astype(BF16)
    y = jnp.broadcast_to(b2, (B, D))
    for i, (r, n) in enumerate(zip(starts, W2_PARTS)):
        wait(w2_v.at[pl.ds(r, n), :], w2sem.at[i])
        y = y + jnp.dot(u[:, r:r + n], w2_v[r:r + n, :], preferred_element_type=F32)
    out_ref[...] = (x1 + gb * y).astype(out_ref.dtype)


@jax.jit
def pallas_adaLN_cond__sliding_block_cached__dense_activation_gelu__decode_kernel(
    A_x: jax.Array,
    A_k_cache: jax.Array,
    A_v_cache: jax.Array,
    A_wq: jax.Array,
    A_wo: jax.Array,
    B_x: jax.Array,
    B_w1: jax.Array,
    B_b1: jax.Array,
    B_w2: jax.Array,
    B_b2: jax.Array,
    c: jax.Array,
    w_mod: jax.Array,
):
    del B_x
    B, Sq, D = A_x.shape
    _, H, Sk, Dh = A_k_cache.shape
    F = B_w1.shape[1]
    W = min(4096, max(256, Sk // 4))
    HD = H * Dh
    assert Sq == 1 and A_wq.shape == (D, HD) and sum(W2_PARTS) == F

    dma = pltpu.SemaphoreType.DMA
    out = pl.pallas_call(
        _block_kernel,
        in_specs=[pl.BlockSpec(memory_space=pltpu.HBM)] * 11,
        out_specs=pl.BlockSpec(memory_space=pltpu.VMEM),
        out_shape=jax.ShapeDtypeStruct((B, D), A_x.dtype),
        scratch_shapes=[
            pltpu.VMEM((B, D), BF16), pltpu.VMEM((B, D), BF16),
            pltpu.VMEM((F,), BF16), pltpu.VMEM((D,), BF16),
            pltpu.VMEM((D, 6 * D), BF16), pltpu.VMEM((D, HD), BF16), pltpu.VMEM((HD, D), BF16),
            pltpu.VMEM((F, D), BF16), pltpu.VMEM((F, D), BF16),
            pltpu.VMEM((B, W, Dh), BF16), pltpu.VMEM((B, W, Dh), BF16),
            pltpu.VMEM((H, B, Dh), F32), pltpu.VMEM((H, B, Dh), F32),
            dma((B,)), dma((B,)), dma((4,)), dma((2,)), dma((Q_PARTS,)), dma(()), dma(()),
            dma((len(W2_PARTS),)),
        ],
        compiler_params=pltpu.CompilerParams(vmem_limit_bytes=64 * 1024 * 1024),
    )(A_x.reshape(B, D), c, w_mod, A_wq, A_k_cache, A_v_cache, A_wo, B_w1.T, B_b1, B_w2, B_b2)
    return out.reshape(B, Sq, D)
```

```python
import jax
import jax.numpy as jnp
from jax import lax
import jax.experimental.pallas as pl
import jax.experimental.pallas.tpu as pltpu

F32 = jnp.float32
BF16 = jnp.bfloat16
_NT = (((1,), (1,)), ((), ()))

KV_ROWS = (128, 64, 64)
IN_ROWS = (8, 8, 8, 8)
OUT_ROWS = (16, 16)
O_HEADS = 8
W2_PARTS = (512, 512, 448, 192, 64)


def _layernorm(x):
    m = jnp.mean(x, axis=-1, keepdims=True)
    d = x - m
    v = jnp.mean(d * d, axis=-1, keepdims=True)
    return d / jnp.sqrt(v + 1e-05)


def _loop(lo, hi, f):
    def body(i, carry):
        f(i)
        return carry

    lax.fori_loop(lo, hi, body, 0)


def _stream(src, dst, sem, rows, unroll=False):
    half, period = dst.shape[0] // 2, sum(rows)
    assert 2 * half == dst.shape[0] and half % period == 0 and all(n % 8 == 0 for n in rows)

    def step(i):
        for k, n in enumerate(rows):
            for queue in range(2):
                r = queue * half + i * period + sum(rows[:k])
                if not isinstance(r, int):
                    r = pl.multiple_of(r, 8)
                pltpu.make_async_copy(src.at[pl.ds(r, n), :], dst.at[pl.ds(r, n), :], sem).start(priority=queue)

    if unroll or half == period:
        for i in range(half // period):
            step(i)
    else:
        _loop(0, half // period, step)


def _wait(dst, sem):
    pltpu.make_async_copy(dst, dst, sem).wait()


def _cols(ref, j, n):
    return ref.at[:, pl.ds(pl.multiple_of(j * n, 128), n)]


def _rows(ref, j, n):
    return ref.at[pl.ds(pl.multiple_of(j * n, 128), n), :]


def _block_kernel(x_hbm, c_hbm, wmod_hbm, wq_hbm, k_hbm, v_hbm, wo_hbm, w1t_hbm, b1_hbm, w2_hbm, b2_hbm,
                  out_ref,
                  x_v, c_v, b1_v, b2_v, wmod_v, wq_v, wo_v, w1_v, w2_v, kbuf, vbuf, q_scr, o_scr, mod_scr,
                  ksem, vsem, wsem):
    B, D = x_v.shape
    _, H, Sk, Dh = k_hbm.shape
    W = kbuf.shape[1]
    F = w1_v.shape[0]
    QN = H * Dh // B
    scale = Dh ** (-0.5)

    def start_wq(j):
        _stream(_cols(wq_hbm, j, QN), wq_v.at[j], wsem.at[j], IN_ROWS)

    def start_kv(b, h):
        window = pl.ds(Sk - W, W)
        _stream(k_hbm.at[b, h, window, :], kbuf.at[b], ksem.at[b], KV_ROWS, unroll=True)
        _stream(v_hbm.at[b, h, window, :], vbuf.at[b], vsem.at[b], KV_ROWS, unroll=True)

    pltpu.make_async_copy(c_hbm, c_v, ksem.at[0]).start(priority=0)
    pltpu.make_async_copy(x_hbm, x_v, ksem.at[1]).start(priority=1)
    _loop(0, 3, lambda j: _stream(_cols(wmod_hbm, j, 2 * D), wmod_v.at[j], vsem.at[j], IN_ROWS))
    _loop(0, B // 2, start_wq)

    _wait(c_v, ksem.at[0])
    _wait(x_v, ksem.at[1])
    cf = c_v[...].astype(F32)
    sc = (cf * jax.nn.sigmoid(cf)).astype(BF16)

    def mod_part(j):
        _wait(wmod_v.at[j], vsem.at[j])
        mod = jnp.dot(sc, wmod_v[j], preferred_element_type=F32)
        mod_scr[2 * j] = mod[:, 0:D]
        mod_scr[2 * j + 1] = mod[:, D:2 * D]

    _loop(0, 3, mod_part)
    ha = (_layernorm(x_v[...].astype(F32)) * (1.0 + mod_scr[1]) + mod_scr[0]).astype(BF16)

    _loop(B // 2, B, start_wq)

    def q_part(j):
        start_kv(j, 0)
        _wait(wq_v.at[j], wsem.at[j])
        q = jnp.dot(ha, wq_v[j], preferred_element_type=F32)
        for i in range(QN // Dh):
            q_scr[j * (QN // Dh) + i] = q[:, i * Dh:(i + 1) * Dh]

    _loop(0, B, q_part)

    row = lax.broadcasted_iota(jnp.int32, (B, Dh), 0)

    def attend(t, acc):
        h = t // B
        b = t % B
        _wait(kbuf.at[b], ksem.at[b])
        s = lax.dot_general(q_scr[h].astype(BF16), kbuf[b], _NT, preferred_element_type=F32) * scale
        p = jnp.exp(s - jnp.max(s, axis=-1, keepdims=True))
        denom = jnp.sum(p, axis=-1, keepdims=True)
        _wait(vbuf.at[b], vsem.at[b])
        o = jnp.dot(p.astype(BF16), vbuf[b], preferred_element_type=F32)
        acc = jnp.where(row == b, o / denom, acc)
        o_scr[h] = acc

        @pl.when(h < H - 1)
        def _():
            start_kv(b, h + 1)

        @pl.when(h == H - 1)
        def _():
            _stream(_rows(wo_hbm, b, QN), _rows(wo_v, b, QN), wsem.at[0], OUT_ROWS)

        return acc

    lax.fori_loop(0, H * B, attend, jnp.zeros((B, Dh), F32))

    pltpu.make_async_copy(b1_hbm, b1_v, wsem.at[2]).start(priority=0)
    pltpu.make_async_copy(b2_hbm, b2_v, wsem.at[3]).start(priority=1)
    _stream(w1t_hbm, w1_v, wsem.at[1], OUT_ROWS)
    _wait(wo_v, wsem.at[0])

    def o_part(j, acc):
        o = jnp.concatenate([o_scr[j * O_HEADS + i] for i in range(O_HEADS)], axis=-1).astype(BF16)
        return acc + jnp.dot(o, _rows(wo_v, j, O_HEADS * Dh)[...], preferred_element_type=F32)

    attn = lax.fori_loop(0, H // O_HEADS, o_part, jnp.zeros((B, D), F32))
    x1 = x_v[...].astype(F32) + mod_scr[2] * attn
    hb = (_layernorm(x1) * (1.0 + mod_scr[4]) + mod_scr[3]).astype(BF16)

    sems = [ksem.at[b] for b in range(B)] + [vsem.at[b] for b in range(B)]
    parts = [(sum(W2_PARTS[:i]), n, sems[i]) for i, n in enumerate(W2_PARTS)]
    for r, n, sem in parts:
        _stream(w2_hbm.at[pl.ds(r, n), :], w2_v.at[pl.ds(r, n), :], sem, OUT_ROWS)
    _wait(b1_v, wsem.at[2])
    _wait(b2_v, wsem.at[3])
    b1 = b1_v[...].astype(F32).reshape(1, F)
    b2 = b2_v[...].astype(F32).reshape(1, D)
    _wait(w1_v, wsem.at[1])
    u = lax.dot_general(hb, w1_v[...], _NT, preferred_element_type=F32) + b1
    u = jax.nn.gelu(u, approximate=True)
    us = [u[:, r:r + n].astype(BF16) for r, n, _ in parts]
    y = jnp.broadcast_to(b2, (B, D))
    for u_part, (r, n, sem) in zip(us, parts):
        _wait(w2_v.at[pl.ds(r, n), :], sem)
        y = y + jnp.dot(u_part, w2_v[r:r + n, :], preferred_element_type=F32)
    out_ref[...] = (x1 + mod_scr[5] * y).astype(out_ref.dtype)


@jax.jit
def pallas_adaLN_cond__sliding_block_cached__dense_activation_gelu__decode_kernel(
    A_x: jax.Array,
    A_k_cache: jax.Array,
    A_v_cache: jax.Array,
    A_wq: jax.Array,
    A_wo: jax.Array,
    B_x: jax.Array,
    B_w1: jax.Array,
    B_b1: jax.Array,
    B_w2: jax.Array,
    B_b2: jax.Array,
    c: jax.Array,
    w_mod: jax.Array,
):
    del B_x
    B, Sq, D = A_x.shape
    _, H, Sk, Dh = A_k_cache.shape
    F = B_w1.shape[1]
    W = min(4096, max(256, Sk // 4))
    HD = H * Dh
    assert (B, Sq) == (4, 1) and A_wq.shape == (D, HD) and sum(W2_PARTS) == F
    assert H % O_HEADS == 0 and H % B == 0

    out = pl.pallas_call(
        _block_kernel,
        in_specs=[pl.BlockSpec(memory_space=pltpu.HBM)] * 11,
        out_specs=pl.BlockSpec(memory_space=pltpu.VMEM),
        out_shape=jax.ShapeDtypeStruct((B, D), A_x.dtype),
        scratch_shapes=[
            pltpu.VMEM((B, D), BF16), pltpu.VMEM((B, D), BF16),
            pltpu.VMEM((F,), BF16), pltpu.VMEM((D,), BF16),
            pltpu.VMEM((3, D, 2 * D), BF16), pltpu.VMEM((B, D, HD // B), BF16),
            pltpu.VMEM((HD, D), BF16), pltpu.VMEM((F, D), BF16), pltpu.VMEM((F, D), BF16),
            pltpu.VMEM((B, W, Dh), BF16), pltpu.VMEM((B, W, Dh), BF16),
            pltpu.VMEM((H, B, Dh), F32), pltpu.VMEM((H, B, Dh), F32),
            pltpu.VMEM((6, B, D), F32),
            pltpu.SemaphoreType.DMA((B,)), pltpu.SemaphoreType.DMA((B,)), pltpu.SemaphoreType.DMA((B,)),
        ],
        compiler_params=pltpu.CompilerParams(vmem_limit_bytes=64 * 1024 * 1024),
    )(A_x.reshape(B, D), c, w_mod, A_wq, A_k_cache, A_v_cache, A_wo, B_w1.T, B_b1, B_w2, B_b2)
    return out.reshape(B, Sq, D)
```
